```python
import jax
import jax.numpy as jnp

def _softmax(x, axis=-1):
    return jax.nn.softmax(x, axis=axis)
def _gelu(x):
    return jax.nn.gelu(x, approximate=True)
def _silu(x):
    return jax.nn.silu(x)
def _sigmoid(x):
    return jax.nn.sigmoid(x)
def _layernorm(x, axis=-1, eps=1e-5):
    m = jnp.mean(x, axis=axis, keepdims=True)
    v = jnp.var(x, axis=axis, keepdims=True)
    return (x - m) / jnp.sqrt(v + eps)
def _scatter_add(tgt, idx, src, axis=0):
    return tgt.at[idx].add(src)
def _segment_sum(src, seg, n):
    return jax.ops.segment_sum(src, seg, n)
class _Rng:
    def __init__(self, key):
        self._k = key
    def _next(self):
        self._k, sub = jax.random.split(self._k)
        return sub
    def normal(self, shape):
        return jax.random.normal(self._next(), shape, dtype=jnp.bfloat16)
    def randint(self, lo, hi, shape):
        return jax.random.randint(self._next(), shape, lo, hi, dtype=jnp.int32)
    def uniform(self, shape, lo=0.0, hi=1.0):
        return jax.random.uniform(self._next(), shape, jnp.bfloat16, lo, hi)
    def permutation(self, n):
        return jax.random.permutation(self._next(), n)


kernel_name = 'standalone__gqa_softmax__near_ridge'

def setup_inputs():
    _rng = _Rng(jax.random.key(int.from_bytes(__import__("os").urandom(4), "little")))
    _w = (lambda a: (lambda t: t.astype(jnp.bfloat16) if jnp.issubdtype(t.dtype, jnp.floating) else t)(jnp.asarray(a)))
    B, Hq, Hkv, Sq, Sk, D = 16, 32, 32, 848, 512, 192
    return {
        "q": _w((lambda *s: _rng.normal(s) * 0.05)(B, Hq, Sq, D)),
        "k": _w((lambda *s: _rng.normal(s) * 0.05)(B, Hkv, Sk, D)),
        "v": _w((lambda *s: _rng.normal(s) * 0.05)(B, Hkv, Sk, D)),
    }

def reference(q, k, v):
    B, Hq, Sq, D = q.shape
    Hkv = k.shape[1]
    rep = Hq // Hkv
    k = jnp.repeat(k, rep, axis=1)
    v = jnp.repeat(v, rep, axis=1)
    scale = D ** -0.5
    scores = jnp.einsum("bhqd,bhkd->bhqk", q, k) * scale
    p = _softmax(scores, axis=-1)
    return jnp.einsum("bhqk,bhkd->bhqd", p, v)
```

```python
import jax, jax.numpy as jnp, numpy as np
import jax.experimental.pallas as pl
import jax.experimental.pallas.tpu as pltpu

def make(hb=2, qc=896, unroll=True):
    def fn(q, k, v):
        B, H, Sq, D = q.shape
        Sk = k.shape[2]
        N = B * H
        qT = jnp.swapaxes(q, 2, 3).reshape(N, D, Sq)
        kT = jnp.swapaxes(k, 2, 3).reshape(N, D, Sk)
        vT = jnp.swapaxes(v, 2, 3).reshape(N, D, Sk)
        c = float(D ** -0.5 * np.log2(np.e))
        chunks = [(s, min(qc, Sq - s)) for s in range(0, Sq, qc)]

        def kern(q_ref, k_ref, v_ref, o_ref):
            def head(h):
                kk = k_ref[h].T
                vv = v_ref[h]
                for (s0, w) in chunks:
                    qq = q_ref[h, :, s0:s0 + w]
                    s = jnp.dot(kk, qq, preferred_element_type=jnp.float32)
                    m = jnp.max(s, axis=0, keepdims=True)
                    p = jnp.exp2((s - m) * c)
                    l = jnp.sum(p, axis=0, keepdims=True)
                    o = jnp.dot(vv, p.astype(jnp.bfloat16), preferred_element_type=jnp.float32)
                    o_ref[h, :, s0:s0 + w] = (o * (1.0 / l)).astype(o_ref.dtype)
            if unroll:
                for h in range(hb):
                    head(h)
            else:
                def body(h, _):
                    head(h)
                    return None
                jax.lax.fori_loop(0, hb, body, None)

        oT = pl.pallas_call(
            kern,
            grid=(N // hb,),
            in_specs=[pl.BlockSpec((hb, D, Sq), lambda i: (i, 0, 0)),
                      pl.BlockSpec((hb, D, Sk), lambda i: (i, 0, 0)),
                      pl.BlockSpec((hb, D, Sk), lambda i: (i, 0, 0))],
            out_specs=pl.BlockSpec((hb, D, Sq), lambda i: (i, 0, 0)),
            out_shape=jax.ShapeDtypeStruct((N, D, Sq), q.dtype),
            compiler_params=pltpu.CompilerParams(dimension_semantics=("parallel",), vmem_limit_bytes=100 * 1024 * 1024),
        )(qT, kT, vT)
        return jnp.swapaxes(oT.reshape(B, H, D, Sq), 2, 3)
    return fn


@jax.jit
def pallas_standalone__gqa_softmax__near_ridge_kernel(q, k, v):
    return make(hb=2, qc=896)(q, k, v)
```

```python
import jax, jax.numpy as jnp, numpy as np
from jax import lax
import jax.experimental.pallas as pl
import jax.experimental.pallas.tpu as pltpu

NT = (((1,), (1,)), ((), ()))

def make(hb=4, chunks=(256, 256, 256, 80), la=1, rem="T", flags=None, sm_first=False):
    def fn(q, k, v):
        B, H, Sq, D = q.shape
        Sk = k.shape[2]
        N = B * H
        qT = jnp.swapaxes(q, 2, 3).reshape(N, D, Sq)
        kT = jnp.swapaxes(k, 2, 3).reshape(N, D, Sk)
        vT = jnp.swapaxes(v, 2, 3).reshape(N, D, Sk)
        c = float(D ** -0.5 * np.log2(np.e))
        assert sum(chunks) == Sq
        starts = np.cumsum((0,) + tuple(chunks[:-1]))
        ch = [(int(s), int(w)) for s, w in zip(starts, chunks)]

        def kern(q_ref, k_ref, v_ref, o_ref):
            units = [(h, s0, w) for h in range(hb) for (s0, w) in ch]
            kcache = {}

            def is_rem(u):
                return rem != "T" and u[2] % 128 != 0

            def qk(u):
                h, s0, w = u
                qq = q_ref[h, :, s0:s0 + w]
                if is_rem(u):
                    return jnp.dot(qq.T, k_ref[h], preferred_element_type=jnp.float32)
                if h not in kcache:
                    kcache[h] = k_ref[h].T
                return jnp.dot(kcache[h], qq, preferred_element_type=jnp.float32)

            def sm(u, s):
                ax = 1 if is_rem(u) else 0
                m = jnp.max(s, axis=ax, keepdims=True)
                p = jnp.exp2((s - m) * c)
                l = jnp.sum(p, axis=ax, keepdims=True)
                r = 1.0 / l
                if is_rem(u) and rem == "N2":
                    return (p * r).astype(jnp.bfloat16), None
                return p.astype(jnp.bfloat16), r

            def pv(u, p, r):
                h, s0, w = u
                if is_rem(u):
                    if rem == "N":
                        o = lax.dot_general(p, v_ref[h], NT, preferred_element_type=jnp.float32)
                        o = (o * r).T
                    else:
                        o = lax.dot_general(v_ref[h], p, NT, preferred_element_type=jnp.float32)
                else:
                    o = jnp.dot(v_ref[h], p, preferred_element_type=jnp.float32) * r
                o_ref[h, :, s0:s0 + w] = o.astype(o_ref.dtype)

            n = len(units)
            S, P = {}, {}
            if la == 1:
                S[0] = qk(units[0])
                for i in range(n):
                    if sm_first:
                        P[i] = sm(units[i], S.pop(i))
                    if i + 1 < n:
                        S[i + 1] = qk(units[i + 1])
                    if not sm_first:
                        P[i] = sm(units[i], S.pop(i))
                    pv(units[i], *P.pop(i))
            else:
                for i in range(n + 2):
                    if i < n:
                        S[i] = qk(units[i])
                    if 0 <= i - 1 < n:
                        P[i - 1] = sm(units[i - 1], S.pop(i - 1))
                    if 0 <= i - 2 < n:
                        pv(units[i - 2], *P.pop(i - 2))

        oT = pl.pallas_call(
            kern,
            grid=(N // hb,),
            in_specs=[pl.BlockSpec((hb, D, Sq), lambda i: (i, 0, 0)),
                      pl.BlockSpec((hb, D, Sk), lambda i: (i, 0, 0)),
                      pl.BlockSpec((hb, D, Sk), lambda i: (i, 0, 0))],
            out_specs=pl.BlockSpec((hb, D, Sq), lambda i: (i, 0, 0)),
            out_shape=jax.ShapeDtypeStruct((N, D, Sq), q.dtype),
            compiler_params=pltpu.CompilerParams(dimension_semantics=("parallel",), vmem_limit_bytes=100 * 1024 * 1024, flags=flags),
        )(qT, kT, vT)
        return jnp.swapaxes(oT.reshape(B, H, D, Sq), 2, 3)
    return fn


@jax.jit
def pallas_standalone__gqa_softmax__near_ridge_kernel(q, k, v):
    return make(hb=8, la=2, chunks=(768, 80), rem='N', flags={'XLA_TPU_FORCE_LP_LLO_SCHEDULER': True})(q, k, v)
```

```python
import jax, jax.numpy as jnp, numpy as np
from jax import lax
import jax.experimental.pallas as pl
import jax.experimental.pallas.tpu as pltpu

NT = (((1,), (1,)), ((), ()))
LP = {'XLA_TPU_FORCE_LP_LLO_SCHEDULER': True}

def make(up=(1, 2, 4, 6, 9, 14), G=16, down=(8, 3, 1), cw=128, la=5, rem="N", flags=LP):
    def fn(q, k, v):
        B, H, Sq, D = q.shape
        Sk = k.shape[2]
        N = B * H
        nmain = (N - sum(up) - sum(down)) // G
        assert nmain * G + sum(up) + sum(down) == N
        sizes = list(up) + [G] * nmain + list(down)
        offs = [int(x) for x in np.cumsum([0] + sizes[:-1])]
        nb = len(sizes)
        Gmax = max(sizes)
        qT = jnp.swapaxes(q, 2, 3).reshape(N, D, Sq)
        kT = jnp.swapaxes(k, 2, 3).reshape(N, D, Sk)
        vT = jnp.swapaxes(v, 2, 3).reshape(N, D, Sk)
        c = float(D ** -0.5 * np.log2(np.e))
        nfull = Sq // 128 * 128
        ch = [(nfull, Sq - nfull)] + [(s, cw) for s in range(0, nfull, cw)]

        def compute(q_ref, k_ref, v_ref, o_ref, nh):
            units = [(h, s0, w) for h in range(nh) for (s0, w) in ch]
            kcache = {}
            is_rem = lambda u: u[2] % 128 != 0

            def qk(i):
                u = units[i]
                h, s0, w = u
                qq = q_ref[h, :, s0:s0 + w]
                if is_rem(u):
                    s = jnp.dot(qq.T, k_ref[h], preferred_element_type=jnp.float32)
                    m = jnp.max(s, axis=1, keepdims=True)
                else:
                    if h not in kcache:
                        kcache[h] = k_ref[h].T
                    s = jnp.dot(kcache[h], qq, preferred_element_type=jnp.float32)
                    m = jnp.max(s, axis=0, keepdims=True)
                return s, m

            def sm(i, s, m):
                u = units[i]
                ax = 1 if is_rem(u) else 0
                p = jnp.exp2((s - m) * c)
                l = jnp.sum(p, axis=ax, keepdims=True)
                r = 1.0 / l
                if is_rem(u) and rem == "N3":
                    p, r = p * r, None
                return p.astype(jnp.bfloat16), r

            def pv(i, p, r):
                u = units[i]
                h, s0, w = u
                if is_rem(u):
                    o = lax.dot_general(p, v_ref[h], NT, preferred_element_type=jnp.float32)
                    o = (o * r).T if rem == "N" else o.astype(o_ref.dtype).T
                else:
                    o = jnp.dot(v_ref[h], p, preferred_element_type=jnp.float32) * r
                o_ref[h, :, s0:s0 + w] = o.astype(o_ref.dtype)

            n = len(units)
            S, P = {}, {}
            for i in range(n + la):
                if i < n:
                    S[i] = qk(i)
                if 0 <= i - 1 < n:
                    P[i - 1] = sm(i - 1, *S.pop(i - 1))
                if 0 <= i - la < n:
                    pv(i - la, *P.pop(i - la))

        def kern(q_hbm, k_hbm, v_hbm, o_hbm, qb, kb, vb, ob, sem):
            def cin(off, n, par):
                return [pltpu.make_async_copy(src.at[pl.ds(off, n)], dst.at[par, pl.ds(0, n)], sem.at[2 * j + par])
                        for j, (src, dst) in enumerate(((q_hbm, qb), (k_hbm, kb), (v_hbm, vb)))]
            def cout(off, n, par):
                return pltpu.make_async_copy(ob.at[par, pl.ds(0, n)], o_hbm.at[pl.ds(off, n)], sem.at[6 + par])
            def start_in(off, n, par):
                for cp in cin(off, n, par): cp.start()

            def static_block(b):
                par = b % 2
                for cp in cin(offs[b], sizes[b], par): cp.wait()
                if b + 1 < nb:
                    start_in(offs[b + 1], sizes[b + 1], 1 - par)
                if b >= 2:
                    cout(offs[b - 2], sizes[b - 2], par).wait()
                compute(qb.at[par], kb.at[par], vb.at[par], ob.at[par], sizes[b])
                cout(offs[b], sizes[b], par).start()

            start_in(0, sizes[0], 0)
            b0 = len(up)
            for b in range(b0):
                static_block(b)

            def body(it, _):
                par = (it + b0) % 2
                off = offs[b0] + it * G
                for cp in cin(off, G, par): cp.wait()
                @pl.when(it < nmain - 1)
                def _(): start_in(off + G, G, 1 - par)
                if b0 + nmain < nb:
                    @pl.when(it == nmain - 1)
                    def _(): start_in(offs[b0 + nmain], sizes[b0 + nmain], (b0 + nmain) % 2)
                for t in range(2):
                    if b0 + t >= 2:
                        @pl.when(it == t)
                        def _(): cout(offs[b0 + t - 2], sizes[b0 + t - 2], (b0 + t) % 2).wait()
                @pl.when(it >= 2)
                def _(): cout(off - 2 * G, G, par).wait()
                compute(qb.at[par], kb.at[par], vb.at[par], ob.at[par], G)
                cout(off, G, par).start()
                return None
            lax.fori_loop(0, nmain, body, None)

            for b in range(b0 + nmain, nb):
                static_block(b)
            for b in range(nb - 2, nb):
                cout(offs[b], sizes[b], b % 2).wait()

        any_spec = pl.BlockSpec(memory_space=pl.ANY)
        oT = pl.pallas_call(
            kern,
            in_specs=[any_spec] * 3,
            out_specs=any_spec,
            out_shape=jax.ShapeDtypeStruct((N, D, Sq), q.dtype),
            scratch_shapes=[pltpu.VMEM((2, Gmax, D, Sq), q.dtype), pltpu.VMEM((2, Gmax, D, Sk), q.dtype),
                            pltpu.VMEM((2, Gmax, D, Sk), q.dtype), pltpu.VMEM((2, Gmax, D, Sq), q.dtype),
                            pltpu.SemaphoreType.DMA((8,))],
            compiler_params=pltpu.CompilerParams(vmem_limit_bytes=110 * 1024 * 1024, flags=flags),
        )(qT, kT, vT)
        return jnp.swapaxes(oT.reshape(B, H, D, Sq), 2, 3)
    return fn


@jax.jit
def pallas_standalone__gqa_softmax__near_ridge_kernel(q, k, v):
    return make(up=(2, 4), G=8, down=(2,))(q, k, v)
```

```python
import jax, jax.numpy as jnp, numpy as np
from jax import lax
import jax.experimental.pallas as pl
import jax.experimental.pallas.tpu as pltpu

NT = (((1,), (1,)), ((), ()))
LP = {'XLA_TPU_FORCE_LP_LLO_SCHEDULER': True}
f32, bf16, u32 = jnp.float32, jnp.bfloat16, jnp.uint32

def make(U=6, G=8, Dn=1, rem="N", flags=LP, nobc=True, prog=0, rempos=1, ktc=True, lead=1):
    def fn(q, k, v):
        B, H, Sq, D = q.shape
        Sk = k.shape[2]
        N = B * H
        M = (N - 1 - U - Dn) // G
        assert 1 + U + M * G + Dn == N
        qT = jnp.swapaxes(q, 2, 3).reshape(N, D, Sq)
        kT = jnp.swapaxes(k, 2, 3).reshape(N, D, Sk)
        vT = jnp.swapaxes(v, 2, 3).reshape(N, D, Sk)
        c = float(D ** -0.5 * np.log2(np.e))
        nfull = Sq // 128 * 128
        wr = Sq - nfull
        ch = [(s, 128) for s in range(0, nfull, 128)]
        ch.insert(rempos, (nfull, wr))
        nu = len(ch)
        is_rem = lambda j: ch[j][1] != 128
        X = 1 if ktc else 0

        def block(q_ref, k_ref, v_ref, o_ref, carry, nh, has_in, has_tail):
            s_c, m_c, kt_c = carry
            kcache = {}
            if has_in and ktc and nh:
                kcache[0] = pltpu.bitcast(kt_c[...], bf16)

            def qk(t, j):
                s0, w = ch[j]
                qq = q_ref[t, :, s0:s0 + w]
                if is_rem(j):
                    s = jnp.dot(qq.T, k_ref[t], preferred_element_type=f32)
                    return s, jnp.max(s, axis=1, keepdims=True)
                if t not in kcache:
                    kcache[t] = k_ref[t].T
                s = jnp.dot(kcache[t], qq, preferred_element_type=f32)
                return s, jnp.max(s, axis=0, keepdims=True)

            def smpv(t, j, s, m):
                s0, w = ch[j]
                p = jnp.exp2((s - m) * c)
                r = 1.0 / jnp.sum(p, axis=1 if is_rem(j) else 0, keepdims=True)
                if is_rem(j) and rem in ("N3", "N5"):
                    p, r = p * r, None
                p = p.astype(bf16)
                if is_rem(j):
                    if rem == "N5":
                        lo = lax.dot_general(p, v_ref[t, :128, :], NT, preferred_element_type=f32)
                        o_ref[t, :128, s0:s0 + w] = lo.astype(bf16).T
                        hi = lax.dot_general(v_ref[t, 128:, :], p, NT, preferred_element_type=f32)
                        o_ref[t, 128:, s0:s0 + w] = hi.astype(bf16)
                        return
                    o = lax.dot_general(p, v_ref[t], NT, preferred_element_type=f32)
                    o = (o * r).T if rem == "N" else o.astype(bf16).T
                else:
                    o = jnp.dot(v_ref[t], p, preferred_element_type=f32) * r
                o_ref[t, :, s0:s0 + w] = o.astype(bf16)

            n = nu * nh
            S = {}
            if has_in:
                for j in range(nu):
                    S[j - nu] = (s_c[j][...], m_c[j][...])
            lag = nu + lead - 1
            for i in range(n + lag + 1):
                if i < n:
                    S[i] = qk(*divmod(i, nu))
                ip = i - lag
                if ip in S and (has_tail or ip < n - nu):
                    t, j = divmod(ip, nu)
                    smpv(t + 1 if has_in else t, j, *S.pop(ip))
            if not has_tail:
                for j in range(nu):
                    s, m = S.pop(n - nu + j)
                    s_c[j][...] = s
                    m_c[j][...] = m
                if ktc:
                    kt_c[...] = pltpu.bitcast(k_ref[nh].T, u32)
            assert not S

        def kern(q_hbm, k_hbm, v_hbm, o_hbm, qa, ka, va, oa, qb, kb, vb, ob, sem_up, sem, *cs):
            carry = (cs[:nu], cs[nu:2 * nu], cs[-1])
            cp = pltpu.make_async_copy

            def up_in(t):
                r = [cp(q_hbm.at[t], qa.at[t], sem_up.at[t]), cp(k_hbm.at[t + X], ka.at[t + X], sem_up.at[t])]
                if not (isinstance(t, int) and t == 0):
                    r.append(cp(v_hbm.at[t - 1], va.at[t], sem_up.at[t]))
                elif X:
                    r.append(cp(k_hbm.at[0], ka.at[0], sem_up.at[0]))
                return r
            def main_in(t0, par):
                return [cp(q_hbm.at[pl.ds(t0, G)], qb.at[par], sem.at[par]),
                        cp(k_hbm.at[pl.ds(t0, G + X)], kb.at[par], sem.at[par]),
                        cp(v_hbm.at[pl.ds(t0 - 1, G)], vb.at[par], sem.at[par])]
            def main_out(t0, par):
                return cp(ob.at[par], o_hbm.at[pl.ds(t0 - 1, G)], sem.at[2 + par])
            tl = 1 + U + M * G
            last_in = [cp(v_hbm.at[pl.ds(tl - 1, Dn + 1)], va.at[pl.ds(0, Dn + 1)], sem.at[4])]
            if Dn:
                last_in += [cp(q_hbm.at[pl.ds(tl, Dn)], qa.at[pl.ds(0, Dn)], sem.at[4]),
                            cp(k_hbm.at[pl.ds(tl, Dn)], ka.at[pl.ds(0, Dn)], sem.at[4])]
            up_out = cp(oa.at[pl.ds(1, U)], o_hbm.at[pl.ds(0, U)], sem.at[5])
            last_out = cp(oa.at[pl.ds(0, Dn + 1)], o_hbm.at[pl.ds(tl - 1, Dn + 1)], sem.at[5])
            def start(cps):
                for x in cps: x.start()
            def wait(cps):
                for x in cps: x.wait()

            if prog == 0:
                for t in range(U + 1):
                    start(up_in(t))
                start(main_in(1 + U, 0))
                wait(up_in(0))
            else:
                start(up_in(0))
                wait(up_in(0))
                for t in range(1, min(prog, U) + 1):
                    start(up_in(t))
            block(qa, ka, va, oa, carry, 1, False, False)

            def up_body(t, _):
                wait(up_in(t))
                if prog:
                    for e in range(2):
                        tn = prog + 1 + 2 * (t - 1) + e
                        @pl.when(tn <= U)
                        def _(): start(up_in(tn))
                        @pl.when(tn == U + 1)
                        def _(): start(main_in(1 + U, 0))
                s = pl.ds(t, 1)
                block(qa.at[s], ka.at[pl.ds(t, 1 + X)], va.at[s], oa.at[s], carry, 1, True, False)
            lax.fori_loop(1, U + 1, up_body, None)

            def main_body(it, _):
                par = it % 2
                t0 = 1 + U + it * G
                wait(main_in(t0, par))
                @pl.when(it < M - 1)
                def _(): start(main_in(t0 + G, 1 - par))
                @pl.when(it == M - 1)
                def _(): start(last_in)
                @pl.when(it == 0)
                def _(): up_out.start()
                @pl.when(it >= 2)
                def _(): main_out(t0 - 2 * G, par).wait()
                block(qb.at[par], kb.at[par], vb.at[par], ob.at[par], carry, G, True, False)
                main_out(t0, par).start()
            lax.fori_loop(0, M, main_body, None)

            wait(last_in)
            up_out.wait()
            block(qa, ka, va, oa, carry, Dn, True, True)
            last_out.start()
            for it in (M - 2, M - 1):
                main_out(1 + U + it * G, it % 2).wait()
            last_out.wait()

        any_spec = pl.BlockSpec(memory_space=pl.ANY)
        A = max(U, Dn) + 1
        V = pltpu.VMEM
        carry_shapes = ([V((wr, Sk), f32) if is_rem(j) else V((Sk, 128), f32) for j in range(nu)]
                        + [V((wr, 1), f32) if is_rem(j) else V((1, 128), f32) for j in range(nu)]
                        + [V((Sk // 2, D), u32)])
        oT = pl.pallas_call(
            kern,
            in_specs=[any_spec] * 3,
            out_specs=any_spec,
            out_shape=jax.ShapeDtypeStruct((N, D, Sq), q.dtype),
            scratch_shapes=[V((A, D, Sq), bf16), V((A + X, D, Sk), bf16), V((A, D, Sk), bf16), V((A, D, Sq), bf16),
                            V((2, G, D, Sq), bf16), V((2, G + X, D, Sk), bf16), V((2, G, D, Sk), bf16), V((2, G, D, Sq), bf16),
                            pltpu.SemaphoreType.DMA((U + 1,)), pltpu.SemaphoreType.DMA((6,))] + carry_shapes,
            compiler_params=pltpu.CompilerParams(vmem_limit_bytes=110 * 1024 * 1024, flags=flags, disable_bounds_checks=nobc),
        )(qT, kT, vT)
        return jnp.swapaxes(oT.reshape(B, H, D, Sq), 2, 3)
    return fn


@jax.jit
def pallas_standalone__gqa_softmax__near_ridge_kernel(q, k, v):
    return make(rem='N5')(q, k, v)
```

```python
import jax
import jax.numpy as jnp
import numpy as np
from jax import lax
import jax.experimental.pallas as pl
import jax.experimental.pallas.tpu as pltpu

_LANES = 128
_RAMP_UP = 13
_BLOCK = 17
_RAMP_DOWN = 5
_LOADS_AHEAD = 2
_LOADS_PER_STEP = 4
_RAGGED_POS = 1
_MIN_LAG = 5
_NT = (((1,), (1,)), ((), ()))


def _compute_block(q_ref, k_ref, v_ref, o_ref, carry, *, units, steps, first, last):
    s_carry, m_carry, k_carry = carry
    n_units = len(units)
    dtype = o_ref.dtype
    log2_scale = float(q_ref.shape[1] ** -0.5 * np.log2(np.e))

    keys = {}
    if steps and not first:
        keys[0] = pltpu.bitcast(k_carry[...], dtype)

    def scores(t, j):
        start, width = units[j]
        qt = q_ref[t, :, start:start + width]
        if width != _LANES:
            s = jnp.dot(qt.T, k_ref[t], preferred_element_type=jnp.float32)
            return s, jnp.max(s, axis=1, keepdims=True)
        if t not in keys:
            keys[t] = k_ref[t].T
        s = jnp.dot(keys[t], qt, preferred_element_type=jnp.float32)
        return s, jnp.max(s, axis=0, keepdims=True)

    def output(t, j, s, m):
        start, width = units[j]
        cols = slice(start, start + width)
        p = jnp.exp2((s - m) * log2_scale)
        if width != _LANES:
            p = (p * (1.0 / jnp.sum(p, axis=1, keepdims=True))).astype(dtype)
            split = v_ref.shape[1] // _LANES * _LANES
            lo = lax.dot_general(p, v_ref[t, :split, :], _NT, preferred_element_type=jnp.float32)
            o_ref[t, :split, cols] = lo.astype(dtype).T
            hi = lax.dot_general(v_ref[t, split:, :], p, _NT, preferred_element_type=jnp.float32)
            o_ref[t, split:, cols] = hi.astype(dtype)
        else:
            inv = 1.0 / jnp.sum(p, axis=0, keepdims=True)
            o = jnp.dot(v_ref[t], p.astype(dtype), preferred_element_type=jnp.float32)
            o_ref[t, :, cols] = (o * inv).astype(dtype)

    n = n_units * steps
    pending = {}
    if not first:
        for j in range(n_units):
            pending[j - n_units] = (s_carry[j][...], m_carry[j][...])
    done = 0 if first else -n_units
    stop = n if last else n - n_units
    for i in range(n + 2 * n_units):
        if i < n:
            pending[i] = scores(*divmod(i, n_units))
        while done <= i - max(_MIN_LAG, n_units - i // 2) and done < stop:
            t, j = divmod(done, n_units)
            output(t + 1, j, *pending.pop(done))
            done += 1
    if not last:
        for j in range(n_units):
            s_carry[j][...], m_carry[j][...] = pending.pop(stop + j)
        k_carry[...] = pltpu.bitcast(k_ref[steps].T, jnp.uint32)
    assert not pending


def _kernel(q_hbm, k_hbm, v_hbm, o_hbm,
            q_ramp, k_ramp, v_ramp, o_ramp, q_main, k_main, v_main, o_main,
            ramp_sem, sem, *carry_refs, units, n_main):
    n_units = len(units)
    carry = (carry_refs[:n_units], carry_refs[n_units:2 * n_units], carry_refs[-1])
    main_start = 1 + _RAMP_UP
    down_start = main_start + n_main * _BLOCK
    copy = pltpu.make_async_copy

    def start(copies):
        for c in copies:
            c.start()

    def wait(copies):
        for c in copies:
            c.wait()

    def up_in(t):
        return [copy(q_hbm.at[t], q_ramp.at[t], ramp_sem.at[t]),
                copy(k_hbm.at[t + 1], k_ramp.at[t + 1], ramp_sem.at[t]),
                copy(v_hbm.at[t - 1], v_ramp.at[t], ramp_sem.at[t])]

    def up_out():
        return copy(o_ramp.at[pl.ds(1, _RAMP_UP)], o_hbm.at[pl.ds(0, _RAMP_UP)], sem.at[5])

    def main_in(t, slot):
        return [copy(q_hbm.at[pl.ds(t, _BLOCK)], q_main.at[slot], sem.at[slot]),
                copy(k_hbm.at[pl.ds(t, _BLOCK + 1)], k_main.at[slot], sem.at[slot]),
                copy(v_hbm.at[pl.ds(t - 1, _BLOCK)], v_main.at[slot], sem.at[slot])]

    def main_out(t, slot):
        return copy(o_main.at[slot], o_hbm.at[pl.ds(t - 1, _BLOCK)], sem.at[2 + slot])

    def down_in():
        n = _RAMP_DOWN
        return [copy(q_hbm.at[pl.ds(down_start, n)], q_ramp.at[pl.ds(0, n)], sem.at[4]),
                copy(k_hbm.at[pl.ds(down_start, n)], k_ramp.at[pl.ds(0, n)], sem.at[4]),
                copy(v_hbm.at[pl.ds(down_start - 1, n + 1)], v_ramp.at[pl.ds(0, n + 1)], sem.at[4])]

    def down_out(i):
        return copy(o_ramp.at[i], o_hbm.at[down_start - 1 + i], ramp_sem.at[i])

    def ramp_step(i):
        one = pl.ds(i, 1)
        _compute_block(q_ramp.at[one], k_ramp.at[pl.ds(i, 2)], v_ramp.at[one], o_ramp.at[one],
                       carry, units=units, steps=1, first=False, last=False)

    first_in = [copy(q_hbm.at[0], q_ramp.at[0], ramp_sem.at[0]),
                copy(k_hbm.at[pl.ds(0, 2)], k_ramp.at[pl.ds(0, 2)], ramp_sem.at[0])]
    start(first_in)
    wait(first_in)
    for t in range(1, _LOADS_AHEAD + 1):
        start(up_in(t))
    _compute_block(q_ramp, k_ramp, v_ramp, o_ramp, carry,
                   units=units, steps=1, first=True, last=False)

    @pl.loop(1, main_start)
    def _(t):
        wait(up_in(t))
        for e in range(_LOADS_PER_STEP):
            ahead = _LOADS_AHEAD + 1 + _LOADS_PER_STEP * (t - 1) + e
            pl.when(ahead < main_start)(lambda: start(up_in(ahead)))
            pl.when(ahead == main_start)(lambda: start(main_in(main_start, 0)))
        ramp_step(t)

    up_out().start()

    @pl.loop(0, n_main)
    def _(i):
        slot = i % 2
        t = main_start + i * _BLOCK
        wait(main_in(t, slot))
        pl.when(i < n_main - 1)(lambda: start(main_in(t + _BLOCK, 1 - slot)))
        pl.when(i == n_main - 1)(lambda: start(down_in()))
        pl.when(i >= 2)(lambda: main_out(t - 2 * _BLOCK, slot).wait())
        _compute_block(q_main.at[slot], k_main.at[slot], v_main.at[slot], o_main.at[slot],
                       carry, units=units, steps=_BLOCK, first=False, last=False)
        main_out(t, slot).start()

    wait(down_in())
    up_out().wait()

    @pl.loop(0, _RAMP_DOWN)
    def _(i):
        ramp_step(i)
        down_out(i).start()

    one = pl.ds(_RAMP_DOWN, 1)
    _compute_block(q_ramp.at[one], k_ramp.at[one], v_ramp.at[one], o_ramp.at[one],
                   carry, units=units, steps=0, first=False, last=True)
    down_out(_RAMP_DOWN).start()
    for i in (n_main - 2, n_main - 1):
        main_out(main_start + i * _BLOCK, i % 2).wait()
    for i in range(_RAMP_DOWN + 1):
        down_out(i).wait()


@jax.jit
def pallas_standalone__gqa_softmax__near_ridge_kernel(
    q: jax.Array,
    k: jax.Array,
    v: jax.Array,
):
    batch, heads, sq, d = q.shape
    sk = k.shape[2]
    n = batch * heads
    n_main, leftover = divmod(n - 1 - _RAMP_UP - _RAMP_DOWN, _BLOCK)
    assert k.shape == v.shape == (batch, heads, sk, d)
    assert leftover == 0 and n_main >= 2 and 1 <= _RAMP_DOWN <= _RAMP_UP
    assert q.dtype == k.dtype == v.dtype == jnp.bfloat16

    aligned = sq // _LANES * _LANES
    units = [(s, _LANES) for s in range(0, aligned, _LANES)]
    units.insert(_RAGGED_POS, (aligned, sq - aligned))

    def vmem(*shape, dtype=q.dtype):
        return pltpu.VMEM(shape, dtype)

    slots = _RAMP_UP + 1
    scratch = [
        vmem(slots, d, sq), vmem(slots + 1, d, sk), vmem(slots, d, sk), vmem(slots, d, sq),
        vmem(2, _BLOCK, d, sq), vmem(2, _BLOCK + 1, d, sk), vmem(2, _BLOCK, d, sk), vmem(2, _BLOCK, d, sq),
        pltpu.SemaphoreType.DMA((slots,)), pltpu.SemaphoreType.DMA((6,)),
    ]
    scratch += [vmem(*((sk, w) if w == _LANES else (w, sk)), dtype=jnp.float32) for _, w in units]
    scratch += [vmem(*((1, w) if w == _LANES else (w, 1)), dtype=jnp.float32) for _, w in units]
    scratch += [vmem(sk // 2, d, dtype=jnp.uint32)]

    def kernel(*refs):
        _kernel(*refs, units=units, n_main=n_main)

    in_hbm = pl.BlockSpec(memory_space=pl.ANY)
    out_t = pl.pallas_call(
        kernel,
        in_specs=[in_hbm] * 3,
        out_specs=in_hbm,
        out_shape=jax.ShapeDtypeStruct((n, d, sq), q.dtype),
        scratch_shapes=scratch,
        compiler_params=pltpu.CompilerParams(
            vmem_limit_bytes=100 * 1024 * 1024,
            disable_bounds_checks=True,
            flags={"XLA_TPU_FORCE_LP_LLO_SCHEDULER": True},
        ),
    )(
        jnp.swapaxes(q, 2, 3).reshape(n, d, sq),
        jnp.swapaxes(k, 2, 3).reshape(n, d, sk),
        jnp.swapaxes(v, 2, 3).reshape(n, d, sk),
    )
    return jnp.swapaxes(out_t.reshape(batch, heads, d, sq), 2, 3)
```
